```python
import os as _os
_os.environ.setdefault("JAX_PLATFORMS", "cpu")
import jax
import jax.numpy as jnp

def _softmax(x, axis=-1):
    return jax.nn.softmax(x, axis=axis)
def _gelu(x):
    return jax.nn.gelu(x, approximate=True)
def _silu(x):
    return jax.nn.silu(x)
def _sigmoid(x):
    return jax.nn.sigmoid(x)
def _layernorm(x, axis=-1, eps=1e-5):
    m = jnp.mean(x, axis=axis, keepdims=True)
    v = jnp.var(x, axis=axis, keepdims=True)
    return (x - m) / jnp.sqrt(v + eps)
def _scatter_add(tgt, idx, src, axis=0):
    return tgt.at[idx].add(src)
def _segment_sum(src, seg, n):
    return jax.ops.segment_sum(src, seg, n)
class _Rng:
    def __init__(self, key):
        self._k = key
    def _next(self):
        self._k, sub = jax.random.split(self._k)
        return sub
    def normal(self, shape):
        return jax.random.normal(self._next(), shape, dtype=jnp.bfloat16)
    def randint(self, lo, hi, shape):
        return jax.random.randint(self._next(), shape, lo, hi, dtype=jnp.int32)
    def uniform(self, shape, lo=0.0, hi=1.0):
        return jax.random.uniform(self._next(), shape, jnp.bfloat16, lo, hi)
    def permutation(self, n):
        return jax.random.permutation(self._next(), n)


kernel_name = 'recurrent_scan__grouped_kv_mqa__mixer_s_mlp__prompt'

def setup_inputs():
    _rng = _Rng(jax.random.key(int.from_bytes(__import__("os").urandom(4), "little")))
    _w = (lambda a: (lambda t: t.astype(jnp.bfloat16) if jnp.issubdtype(t.dtype, jnp.floating) else t)(jnp.asarray(a)))
    def _A_setup():
        B, S, D, H = 1, 2048, 512, 32
        Dh = D // H
        return {
            "x": _w((lambda *s: _rng.normal(s) * 0.05)(B, S, D)),
            "wq": _w((lambda *s: _rng.normal(s) * 0.05)(D, H * Dh)),
            "wk": _w((lambda *s: _rng.normal(s) * 0.05)(D, Dh)),
            "wv": _w((lambda *s: _rng.normal(s) * 0.05)(D, Dh)),
            "wo": _w((lambda *s: _rng.normal(s) * 0.05)(H * Dh, D)),
        }
    _A_in = _A_setup()

    def _B_setup():
        B, S, D, F = 1, 2048, 512, 1792
        return {
            "x":  _w((lambda *s: _rng.normal(s) * 0.05)(B, S, D)),
            "w1": _w((lambda *s: _rng.normal(s) * 0.8)(D, D) * (D ** -0.5)),
            "w2": _w((lambda *s: _rng.normal(s) * 0.8)(D, D) * (D ** -0.5)),
            "w3": _w((lambda *s: _rng.normal(s) * 0.8)(D, F) * (D ** -0.5)),
            "w4": _w((lambda *s: _rng.normal(s) * 0.8)(F, D) * (F ** -0.5)),
        }
    _B_in = _B_setup()

    return {
        "A_x": _A_in["x"],
        "A_wq": _A_in["wq"],
        "A_wk": _A_in["wk"],
        "A_wv": _A_in["wv"],
        "A_wo": _A_in["wo"],
        "B_x": _B_in["x"],
        "B_w1": _B_in["w1"],
        "B_w2": _B_in["w2"],
        "B_w3": _B_in["w3"],
        "B_w4": _B_in["w4"],
    }

def reference(A_x, A_wq, A_wk, A_wv, A_wo, B_x, B_w1, B_w2, B_w3, B_w4):
    def _A_ref(x, wq, wk, wv, wo):
        B, S, D = x.shape
        H = 32
        Dh = D // H
        q = (lambda x, *d: x.transpose(*d))((x @ wq).reshape(B, S, H, Dh), 0, 2, 1, 3)
        k = x @ wk
        v = x @ wv
        scores = jnp.einsum("bhqd,bkd->bhqk", q, k) * (Dh ** -0.5)
        p = _softmax(scores, axis=-1)
        o = jnp.einsum("bhqk,bkd->bhqd", p, v)
        return (lambda x, *d: x.transpose(*d))(o, 0, 2, 1, 3).reshape(B, S, H * Dh) @ wo

    def _B_ref(x, w1, w2, w3, w4):
        B, S, D = x.shape
        h = _gelu(_layernorm(x, axis=-1) @ w1)
        c = D // 4
        g0 = jnp.pad(h[:, :, 0*c:1*c], ((0, 0), (1, 0), (0, 0)))[:, :S, :]
        g1 = jnp.pad(h[:, :, 1*c:2*c], ((0, 0), (0, 1), (0, 0)))[:, 1:, :]
        g2 = jnp.pad(h[:, :, 2*c:3*c], ((0, 0), (2, 0), (0, 0)))[:, :S, :]
        g3 = jnp.pad(h[:, :, 3*c:   ], ((0, 0), (0, 2), (0, 0)))[:, 2:, :]
        hs = jnp.concatenate([g0, g1, g2, g3], axis=-1) @ w2
        x1 = x + hs
        h2 = _gelu(_layernorm(x1, axis=-1) @ w3) @ w4
        return x1 + h2

    x = A_x
    xn = _layernorm(x, axis=-1)
    s = _A_ref(xn, A_wq, A_wk, A_wv, A_wo)
    g = _silu(_B_ref(xn, B_w1, B_w2, B_w3, B_w4))
    return x + s * g
```

```python
import functools
import math
import jax
import jax.numpy as jnp
import numpy as np
import jax.experimental.pallas as pl
import jax.experimental.pallas.tpu as pltpu

_BF = jnp.bfloat16
_F32 = jnp.float32
_NT = (((1,), (1,)), ((), ()))
_TN = (((0,), (0,)), ((), ()))

S, D, H, DH, F = 2048, 512, 32, 16, 1792
TQ = 512
TK = 256
U = 4
PAD = 8
L_SAFE = 2.0 ** -24


def _ln(x):
    m = jnp.mean(x, axis=-1, keepdims=True)
    c = x - m
    v = jnp.mean(c * c, axis=-1, keepdims=True)
    return c * jax.lax.rsqrt(v + 1e-5)


def _gelu(x):
    t = jnp.tanh(math.sqrt(2.0 / math.pi) * (x + 0.044715 * (x * x * x)))
    return 0.5 * x * (1.0 + t)


def _dot(a, b, dims=None):
    if dims is None:
        return jnp.dot(a, b, preferred_element_type=_F32)
    return jax.lax.dot_general(a, b, dims, preferred_element_type=_F32)


def _kernel(x_hbm, wq_hbm, wk_hbm, wv_hbm, wo_hbm, w1_hbm, w2_hbm, w3_hbm, w4_hbm, o_ref,
            x_s, wq_s, wkv_s, wo_s, w1_s, w2_s, w3_s, w4_s,
            xn_s, h_s, qe_s, ke_s, vt_s, ot_s, lmin_s, sems):
    i = pl.program_id(0)
    nb = S // TQ

    def cp(n):
        src, dst = {
            "x0": (x_hbm.at[0, pl.ds(0 * TQ, TQ)], x_s.at[pl.ds(0 * TQ, TQ)]),
            "x1": (x_hbm.at[0, pl.ds(1 * TQ, TQ)], x_s.at[pl.ds(1 * TQ, TQ)]),
            "x2": (x_hbm.at[0, pl.ds(2 * TQ, TQ)], x_s.at[pl.ds(2 * TQ, TQ)]),
            "x3": (x_hbm.at[0, pl.ds(3 * TQ, TQ)], x_s.at[pl.ds(3 * TQ, TQ)]),
            "wk": (wk_hbm, wkv_s.at[pl.ds(0, DH)]),
            "wv": (wv_hbm, wkv_s.at[pl.ds(DH, DH)]),
            "wq": (wq_hbm, wq_s), "w1": (w1_hbm, w1_s), "w2": (w2_hbm, w2_s),
            "wo": (wo_hbm, wo_s), "w3": (w3_hbm, w3_s), "w4": (w4_hbm, w4_s),
        }[n]
        return pltpu.make_async_copy(src, dst, sems.at[names.index(n)])

    names = ["x0", "wq", "wk", "wv", "w1", "x1", "x2", "x3", "w2", "wo", "w3", "w4"]

    @pl.when(i == 0)
    def _prologue():
        for n in names:
            cp(n).start()
        h_s[pl.ds(0, PAD), :] = jnp.zeros((PAD, D), _F32)
        h_s[pl.ds(PAD + S, PAD), :] = jnp.zeros((PAD, D), _F32)
        cp("wq").wait()
        wqt = wq_s[...].T
        hsel = (jax.lax.broadcasted_iota(jnp.int32, (H, D), 1) // DH
                == jax.lax.broadcasted_iota(jnp.int32, (H, D), 0)).astype(_BF)
        cp("wk").wait()
        cp("wv").wait()
        cp("w1").wait()
        kn = None
        qn = []
        for b in range(nb):
            rows = pl.ds(b * TQ, TQ)
            cp("x%d" % b).wait()
            xn = _ln(x_s[rows, :].astype(_F32)).astype(_BF)
            xn_s[rows, :] = xn
            kvt = _dot(wkv_s[...], xn, _NT).astype(_BF)
            vt_s[:, rows] = kvt[DH:, :]
            kt = kvt[:DH, :].astype(_F32)
            k2 = jnp.max(jnp.sum(kt * kt, axis=0, keepdims=True), axis=1, keepdims=True)
            kn = k2 if kn is None else jnp.maximum(kn, k2)
            row = jax.lax.broadcasted_iota(jnp.int32, (2 * DH, TQ), 0)
            ket = jnp.where(row < DH, kvt.astype(_F32), jnp.where(row == DH, -1.0, 0.0))
            ke_s[rows, :] = ket.T.astype(_BF)
            qt = (_dot(wqt, xn, _NT) * (DH ** -0.5 * math.log2(math.e))).astype(_BF)
            for h in range(H):
                qe_s[b, pl.ds(2 * DH * h, DH), :] = qt[DH * h:DH * (h + 1), :]
            qf = qt.astype(_F32)
            qn.append(_dot(hsel, (qf * qf).astype(_BF)))
            h_s[pl.ds(PAD + b * TQ, TQ), :] = _gelu(_dot(xn, w1_s[...]))
        for b in range(nb):
            mh = jnp.sqrt(qn[b]) * jnp.sqrt(kn) * 1.02
            for h in range(H):
                qe_s[b, pl.ds(2 * DH * h + DH, DH), :] = jnp.broadcast_to(
                    mh[h:h + 1, :], (DH, TQ)).astype(_BF)
        cp("w2").wait()
        cp("wo").wait()
        cp("w3").wait()
        cp("w4").wait()

    nk = S // TK

    def heads(g, lmin):
        qts = [qe_s[i, pl.ds(pl.multiple_of((g * U + u) * 2 * DH, 2 * DH), 2 * DH), :] for u in range(U)]
        accs = [None] * U
        ls = [None] * U
        prev = None
        for t in range(U * nk + 1):
            if t < U * nk:
                u, j = divmod(t, nk)
                s = _dot(ke_s[j * TK:(j + 1) * TK, :], qts[u])
            if prev is not None:
                pu, pj, pp = prev
                a = _dot(vt_s[:, pj * TK:(pj + 1) * TK], pp)
                accs[pu] = a if accs[pu] is None else accs[pu] + a
                if pj == nk - 1:
                    l = jnp.sum(ls[pu], axis=0, keepdims=True)
                    lmin = jnp.minimum(lmin, jnp.where(l >= L_SAFE, 1.0, 0.0))
                    ot_s[pl.ds(pl.multiple_of((g * U + pu) * DH, DH), DH), :] = (
                        accs[pu] * (1.0 / l)).astype(_BF)
            if t < U * nk:
                p = jnp.exp2(s)
                ps = p.reshape(TK // 8, 8, TQ).sum(axis=0)
                ls[u] = ps if ls[u] is None else ls[u] + ps
                prev = (u, j, p.astype(_BF))
        return lmin

    ok = jax.lax.fori_loop(0, H // U, heads, jnp.ones((1, TQ), _F32))

    @pl.when(jnp.min(ok) < 0.5)
    def _fallback():
        def head(h, c):
            qt = qe_s[i, pl.ds(pl.multiple_of(h * 2 * DH, 2 * DH), DH), :]

            def chunk(j, carry):
                m, l, acc = carry
                r = pl.ds(pl.multiple_of(j * TK, TK), TK)
                s = _dot(ke_s[r, :][:, :DH], qt)
                mn = jnp.maximum(m, jnp.max(s, axis=0, keepdims=True))
                p = jnp.exp2(s - mn)
                a = jnp.exp2(m - mn)
                l = a * l + jnp.sum(p, axis=0, keepdims=True)
                acc = a * acc + _dot(vt_s[:, r], p.astype(_BF))
                return mn, l, acc

            m, l, acc = jax.lax.fori_loop(
                0, nk, chunk,
                (jnp.full((1, TQ), -jnp.inf, _F32), jnp.zeros((1, TQ), _F32), jnp.zeros((DH, TQ), _F32)))
            ot_s[pl.ds(pl.multiple_of(h * DH, DH), DH), :] = (acc / l).astype(_BF)
            return c
        jax.lax.fori_loop(0, H, head, 0)

    base = pl.multiple_of(i * TQ, TQ)
    c = D // 4
    hw = h_s[pl.ds(base, TQ + 2 * PAD), :]
    g = jnp.concatenate([
        hw[PAD - 1:PAD - 1 + TQ, 0 * c:1 * c],
        hw[PAD + 1:PAD + 1 + TQ, 1 * c:2 * c],
        hw[PAD - 2:PAD - 2 + TQ, 2 * c:3 * c],
        hw[PAD + 2:PAD + 2 + TQ, 3 * c:4 * c]], axis=1).astype(_BF)
    x1 = xn_s[pl.ds(base, TQ), :].astype(_F32) + _dot(g, w2_s[...])
    y = _ln(x1).astype(_BF)
    h2 = _dot(_gelu(_dot(y, w3_s[...])).astype(_BF), w4_s[...])
    z = x1 + h2
    gate = z * (1.0 / (1.0 + jnp.exp(-z)))
    sattn = _dot(ot_s[...], wo_s[...], _TN)
    o_ref[0] = (x_s[pl.ds(base, TQ), :].astype(_F32) + sattn * gate).astype(o_ref.dtype)


@jax.jit
def pallas_recurrent_scan__grouped_kv_mqa__mixer_s_mlp__prompt_kernel(
        A_x, A_wq, A_wk, A_wv, A_wo, B_x, B_w1, B_w2, B_w3, B_w4):
    any_spec = pl.BlockSpec(memory_space=pl.ANY)
    return pl.pallas_call(
        _kernel,
        grid=(S // TQ,),
        in_specs=[any_spec] * 9,
        out_specs=pl.BlockSpec((1, TQ, D), lambda i: (0, i, 0)),
        out_shape=jax.ShapeDtypeStruct((1, S, D), A_x.dtype),
        scratch_shapes=[
            pltpu.VMEM((S, D), _BF), pltpu.VMEM((D, D), _BF), pltpu.VMEM((2 * DH, D), _BF),
            pltpu.VMEM((D, D), _BF), pltpu.VMEM((D, D), _BF), pltpu.VMEM((D, D), _BF),
            pltpu.VMEM((D, F), _BF), pltpu.VMEM((F, D), _BF),
            pltpu.VMEM((S, D), _BF), pltpu.VMEM((S + 2 * PAD, D), _F32),
            pltpu.VMEM((S // TQ, 2 * DH * H, TQ), _BF), pltpu.VMEM((S, 2 * DH), _BF),
            pltpu.VMEM((DH, S), _BF), pltpu.VMEM((D, TQ), _BF), pltpu.VMEM((8, TQ), _F32),
            pltpu.SemaphoreType.DMA((12,)),
        ],
        compiler_params=pltpu.CompilerParams(
            dimension_semantics=("arbitrary",), vmem_limit_bytes=100 * 2 ** 20),
    )(A_x, A_wq, A_wk.T, A_wv.T, A_wo, B_w1, B_w2, B_w3, B_w4)
```

```python
import math
import jax
import jax.numpy as jnp
import jax.experimental.pallas as pl
import jax.experimental.pallas.tpu as pltpu

_BF = jnp.bfloat16
_F32 = jnp.float32
_NT = (((1,), (1,)), ((), ()))
_TN = (((0,), (0,)), ((), ()))

S, D, H, DH, F = 2048, 512, 32, 16, 1792
TQ = 512
TK = TQ
TS = 32
TP = 128
NV = 224
LAG = 2
PL = 4
W = 7
U = 8
NS = 4
PAD = 8
L_SAFE = 2.0 ** -24


def _ln(x):
    m = jnp.mean(x, axis=-1, keepdims=True)
    c = x - m
    v = jnp.mean(c * c, axis=-1, keepdims=True)
    return c * jax.lax.rsqrt(v + 1e-5)


def _gelu(x):
    t = jnp.tanh(math.sqrt(2.0 / math.pi) * (x + 0.044715 * (x * x * x)))
    return 0.5 * x * (1.0 + t)


def _dot(a, b, dims=None):
    if dims is None:
        return jnp.dot(a, b, preferred_element_type=_F32)
    return jax.lax.dot_general(a, b, dims, preferred_element_type=_F32)


def _pack(p):
    return jnp.concatenate([
        pltpu.pack_elementwise([p[x:x + 8], p[x + 8:x + 16]], packed_dtype=_BF)
        for x in range(0, p.shape[0], 16)], axis=0)


def _kernel(x_hbm, wq_hbm, wk_hbm, wv_hbm, wo_hbm, w1_hbm, w2_hbm, w3_hbm, w4_hbm, o_ref,
            x_s, wq_s, wkv_s, wo_s, w1_s, w2_s, w3_s, w4_s,
            xn_s, h_s, qe_s, qf_s, qn_s, kf_s, ke_s, kb_s, vt_s, ot_s, pv_s, sems):
    i = pl.program_id(0)
    nb = S // TQ

    def cp(n):
        src, dst = {
            "x0": (x_hbm.at[0, pl.ds(0 * TQ, TQ)], x_s.at[pl.ds(0 * TQ, TQ)]),
            "x1": (x_hbm.at[0, pl.ds(1 * TQ, TQ)], x_s.at[pl.ds(1 * TQ, TQ)]),
            "x2": (x_hbm.at[0, pl.ds(2 * TQ, TQ)], x_s.at[pl.ds(2 * TQ, TQ)]),
            "x3": (x_hbm.at[0, pl.ds(3 * TQ, TQ)], x_s.at[pl.ds(3 * TQ, TQ)]),
            "wk": (wk_hbm, wkv_s.at[pl.ds(0, DH)]),
            "wv": (wv_hbm, wkv_s.at[pl.ds(DH, DH)]),
            "wq": (wq_hbm, wq_s), "w1": (w1_hbm, w1_s), "w2": (w2_hbm, w2_s),
            "wo": (wo_hbm, wo_s), "w3": (w3_hbm, w3_s), "w4": (w4_hbm, w4_s),
        }[n]
        return pltpu.make_async_copy(src, dst, sems.at[names.index(n)])

    names = ["x0", "x1", "x2", "x3", "wq", "wk", "wv", "w1", "w2", "wo", "w3", "w4"]

    @pl.when(i == 0)
    def _prologue():
        for n in ("wq", "x0", "w1", "wk", "wv"):
            cp(n).start()
        h_s[pl.ds(0, PAD), :] = jnp.zeros((PAD, D), _F32)
        h_s[pl.ds(PAD + S, PAD), :] = jnp.zeros((PAD, D), _F32)
        cp("wq").wait()
        wqt = wq_s[...].T
        hsel = (jax.lax.broadcasted_iota(jnp.int32, (H, D), 1) // DH
                == jax.lax.broadcasted_iota(jnp.int32, (H, D), 0)).astype(_BF)
        cp("x0").wait()
        xn_s[pl.ds(0, TQ), :] = _ln(x_s[pl.ds(0, TQ), :].astype(_F32)).astype(_BF)
        cp("wk").wait()
        cp("wv").wait()
        cp("w1").wait()
        for n in ("x1", "x2", "x3"):
            cp(n).start()

        def block(b, kn):
            rows = pl.ds(pl.multiple_of(b * TQ, TQ), TQ)
            nxt = pl.ds(pl.multiple_of(jnp.minimum(b + 1, nb - 1) * TQ, TQ), TQ)

            @pl.when(b + 1 < nb)
            def _():
                pltpu.make_async_copy(x_hbm.at[0, nxt], x_s.at[nxt], sems.at[b + 1]).wait()

            xn = xn_s[rows, :]
            hpre = _dot(xn, w1_s[...])
            kvt = _dot(wkv_s[...], xn, _NT).astype(_BF)
            qt = _dot(wqt, xn, _NT)
            h_s[pl.ds(pl.multiple_of(PAD + b * TQ, 8), TQ), :] = _gelu(hpre)
            vt_s[b] = kvt[DH:, :]
            kt = kvt[:DH, :].astype(_F32)
            kn = jnp.maximum(kn, jnp.sum(kt * kt, axis=0, keepdims=True))
            row = jax.lax.broadcasted_iota(jnp.int32, (2 * DH, TQ), 0)
            ket = jnp.where(row < DH, kvt.astype(_F32), jnp.where(row == DH, -1.0, 0.0))
            kf_s[...] = ket.T
            kp = jnp.concatenate([
                kf_s[pl.ds(e, TQ // 2, stride=2), :].reshape(TQ // 16, 8, 2 * DH) for e in range(2)],
                axis=1).reshape(TQ, 2 * DH)
            ke_s[pl.ds(pl.multiple_of(b * (TQ // 2), TQ // 2), TQ // 2), :] = pltpu.bitcast(kp.astype(_BF), jnp.uint32)
            qt = (qt * (DH ** -0.5 * math.log2(math.e))).astype(_BF)
            qf = qt.astype(_F32)
            for h in range(H):
                qe_s[b, pl.ds(2 * DH * h, DH), :] = qt[DH * h:DH * (h + 1), :]
                qf_s[b, h, pl.ds(0, DH), :] = qf[DH * h:DH * (h + 1), :]
            qn_s[b] = _dot(hsel, (qf * qf).astype(_BF))
            xn_s[nxt, :] = _ln(x_s[nxt, :].astype(_F32)).astype(_BF)
            return kn

        kn = jax.lax.fori_loop(0, nb, block, jnp.zeros((1, TQ), _F32))
        for n in ("w2", "wo", "w3", "w4"):
            cp(n).start()
        kmax = jnp.sqrt(jnp.max(kn, axis=1, keepdims=True)) * 1.02
        kv = pltpu.bitcast(ke_s[pl.ds((S - NV) // 2, NV // 2), :], _BF).astype(_F32)
        for d in range(DH):
            kb_s[d] = jnp.broadcast_to(kv[:, d:d + 1], (NV, 128))

        def bound(b, c):
            mh = (jnp.sqrt(qn_s[b]) * kmax).astype(_BF).astype(_F32)
            for h in range(H):
                qe_s[b, pl.ds(2 * DH * h + DH, DH), :] = jnp.broadcast_to(
                    mh[h:h + 1, :], (DH, TQ)).astype(_BF)
                qf_s[b, h, pl.ds(DH, 8), :] = jnp.broadcast_to(-mh[h:h + 1, :], (8, TQ))
            return c
        jax.lax.fori_loop(0, nb, bound, 0)

    nk = S // TK

    ns = (S - NV) // TS
    vwork = [(a, b) for a in range(0, NV, 16) for b in range(0, TQ, 128)]

    def vt(lo, hi):
        return vt_s[lo // TQ, :, lo % TQ:lo % TQ + hi - lo]

    def heads(g, ok):
        qts = [qe_s[i, pl.ds(pl.multiple_of((g * U + u) * 2 * DH, 2 * DH), 2 * DH), :] for u in range(U)]
        accs = [None] * U
        ls = [None] * U
        lv = [{} for _ in range(U)]
        scores, ready, back, pq = {}, {}, {}, []
        never = h_s[0:8, 0:128] > 0.5
        T = U * ns
        for t in range(T + LAG + PL):
            if t < T:
                u, j = divmod(t, ns)
                kw = ke_s[j * TS // 2:(j + 1) * TS // 2, :]
                if t in back:
                    kw = jnp.concatenate([jnp.where(never[:, :2 * DH], back.pop(t), kw[:8]), kw[8:]], axis=0)
                scores[t] = _dot(pltpu.bitcast(kw, _BF), qts[u])
            if t in ready:
                u, j, pp = ready.pop(t)
                e = (j + 1) * TS
                lo = e - 2 * pp.shape[0]
                if j == ns - 1:
                    pp, e = jnp.concatenate([pp, pv_s[u % 2]], axis=0), S
                a = _dot(vt(lo, e), pltpu.bitcast(pp, _BF))
                accs[u] = a if accs[u] is None else accs[u] + a
                if j == ns - 1:
                    acc = accs[u]
                    l = ls[u] + jnp.concatenate([lv[u][b] for b in range(0, TQ, 128)], axis=1)
                    l = jnp.sum(l, axis=0, keepdims=True)
                    ok = jnp.where((l >= L_SAFE) & (l <= 2.0 * S), ok, 0.0)
                    ot_s[pl.ds(pl.multiple_of((g * U + u) * DH, DH), DH), :] = (
                        acc * (1.0 / l)).astype(_BF)
            if LAG <= t < T + LAG:
                u, j = divmod(t - LAG, ns)
                sc = scores.pop(t - LAG)
                p = jnp.exp2(sc)
                ps = p.reshape(TS // 8, 8, TQ).sum(axis=0)
                ls[u] = ps if ls[u] is None else ls[u] + ps
                pq.append(_pack(p))
                if len(pq) == TP // TS or j == ns - 1:
                    ready[t + PL] = (u, j, jnp.concatenate(pq, axis=0))
                    pq = []
                for a, b in vwork[j * len(vwork) // ns:(j + 1) * len(vwork) // ns]:
                    hq = g * U + u
                    sv = jnp.where(never, sc[:8, b:b + 128], qf_s[i, hq, DH:DH + 8, b:b + 128])
                    sv = jnp.concatenate([sv, sv], axis=0)
                    for d in range(DH):
                        sv = sv + kb_s[d, a:a + 16, :] * jnp.broadcast_to(
                            qf_s[i, hq, d:d + 1, b:b + 128], (16, 128))
                    p = jnp.exp2(sv)
                    ps = p[:8] + p[8:]
                    lv[u][b] = lv[u][b] + ps if b in lv[u] else ps
                    pw = _pack(p)
                    pv_s[u % 2, a // 2:a // 2 + 8, b:b + 128] = pw
                    back[t - LAG + W] = pw[:, :2 * DH]
        return ok

    ok = jax.lax.fori_loop(0, H // U, heads, jnp.ones((1, TQ), _F32))

    @pl.when(jnp.min(ok) < 0.5)
    def _fallback():
        def head(h, c):
            qt = qe_s[i, pl.ds(pl.multiple_of(h * 2 * DH, 2 * DH), DH), :]

            def chunk(j, carry):
                m, l, acc = carry
                r = pl.ds(pl.multiple_of(j * (TK // 2), TK // 2), TK // 2)
                s = _dot(pltpu.bitcast(ke_s[r, :], _BF)[:, :DH], qt)
                mn = jnp.maximum(m, jnp.max(s, axis=0, keepdims=True))
                p = jnp.exp2(s - mn)
                a = jnp.exp2(m - mn)
                l = a * l + jnp.sum(p, axis=0, keepdims=True)
                acc = a * acc + _dot(vt_s[j], pltpu.bitcast(_pack(p), _BF))
                return mn, l, acc

            m, l, acc = jax.lax.fori_loop(
                0, nk, chunk,
                (jnp.full((1, TQ), -jnp.inf, _F32), jnp.zeros((1, TQ), _F32), jnp.zeros((DH, TQ), _F32)))
            ot_s[pl.ds(pl.multiple_of(h * DH, DH), DH), :] = (acc / l).astype(_BF)
            return c
        jax.lax.fori_loop(0, H, head, 0)

    @pl.when(i == 0)
    def _():
        cp("w2").wait()
        cp("wo").wait()
        cp("w3").wait()
        cp("w4").wait()

    c = D // 4
    TM = TQ // NS
    parts = range(NS)
    rows = [pl.ds(pl.multiple_of(i * TQ + r * TM, TM), TM) for r in parts]

    def shifted(r):
        hw = h_s[pl.ds(pl.multiple_of(i * TQ + r * TM, TM), TM + 2 * PAD), :]
        return jnp.concatenate([
            hw[PAD - 1:PAD - 1 + TM, 0 * c:1 * c],
            hw[PAD + 1:PAD + 1 + TM, 1 * c:2 * c],
            hw[PAD - 2:PAD - 2 + TM, 2 * c:3 * c],
            hw[PAD + 2:PAD + 2 + TM, 3 * c:4 * c]], axis=1).astype(_BF)

    def attn_out(r):
        return _dot(ot_s[:, r * TM:(r + 1) * TM], wo_s[...], _TN)

    x1 = [xn_s[rows[r], :].astype(_F32) + _dot(shifted(r), w2_s[...]) for r in parts]
    sattn = [attn_out(r) for r in range(NS - 1)]
    up = [_dot(_ln(x1[r]).astype(_BF), w3_s[...]) for r in parts]
    z = [x1[r] + _dot(_gelu(up[r]).astype(_BF), w4_s[...]) for r in parts]
    sattn.append(attn_out(NS - 1))
    for r in parts:
        gate = z[r] * (1.0 / (1.0 + jnp.exp(-z[r])))
        o_ref[0, r * TM:(r + 1) * TM, :] = (
            x_s[rows[r], :].astype(_F32) + sattn[r] * gate).astype(o_ref.dtype)


@jax.jit
def pallas_recurrent_scan__grouped_kv_mqa__mixer_s_mlp__prompt_kernel(
        A_x, A_wq, A_wk, A_wv, A_wo, B_x, B_w1, B_w2, B_w3, B_w4):
    any_spec = pl.BlockSpec(memory_space=pl.ANY)
    return pl.pallas_call(
        _kernel,
        grid=(S // TQ,),
        in_specs=[any_spec] * 9,
        out_specs=pl.BlockSpec((1, TQ, D), lambda i: (0, i, 0)),
        out_shape=jax.ShapeDtypeStruct((1, S, D), A_x.dtype),
        scratch_shapes=[
            pltpu.VMEM((S, D), _BF), pltpu.VMEM((D, D), _BF), pltpu.VMEM((2 * DH, D), _BF),
            pltpu.VMEM((D, D), _BF), pltpu.VMEM((D, D), _BF), pltpu.VMEM((D, D), _BF),
            pltpu.VMEM((D, F), _BF), pltpu.VMEM((F, D), _BF),
            pltpu.VMEM((S, D), _BF), pltpu.VMEM((S + 2 * PAD, D), _F32),
            pltpu.VMEM((S // TQ, 2 * DH * H, TQ), _BF), pltpu.VMEM((S // TQ, H, DH + 8, TQ), _F32),
            pltpu.VMEM((S // TQ, H, TQ), _F32), pltpu.VMEM((TQ, 2 * DH), _F32),
            pltpu.VMEM((S // 2, 2 * DH), jnp.uint32), pltpu.VMEM((DH, NV, 128), _F32),
            pltpu.VMEM((S // TQ, DH, TQ), _BF), pltpu.VMEM((D, TQ), _BF),
            pltpu.VMEM((2, NV // 2, TQ), jnp.uint32),
            pltpu.SemaphoreType.DMA((12,)),
        ],
        compiler_params=pltpu.CompilerParams(
            dimension_semantics=("arbitrary",), vmem_limit_bytes=100 * 2 ** 20),
    )(A_x, A_wq, A_wk.T, A_wv.T, A_wo, B_w1, B_w2, B_w3, B_w4)
```

```python
import math
import jax
import jax.numpy as jnp
import jax.experimental.pallas as pl
import jax.experimental.pallas.tpu as pltpu

_BF = jnp.bfloat16
_F32 = jnp.float32
_NT = (((1,), (1,)), ((), ()))
_TN = (((0,), (0,)), ((), ()))

S, D, H, DH, F = 2048, 512, 32, 16, 1792
TQ = 512
TK = TQ
TS = 32
TP = 128
NV = 224
LAG = 2
PL = 4
W = 7
U = 8
NS = 4
PAD = 8
L_SAFE = 2.0 ** -24


def _ln(x):
    m = jnp.mean(x, axis=-1, keepdims=True)
    c = x - m
    v = jnp.mean(c * c, axis=-1, keepdims=True)
    return c * jax.lax.rsqrt(v + 1e-5)


def _gelu(x):
    t = jnp.tanh(math.sqrt(2.0 / math.pi) * (x + 0.044715 * (x * x * x)))
    return 0.5 * x * (1.0 + t)


def _dot(a, b, dims=None):
    if dims is None:
        return jnp.dot(a, b, preferred_element_type=_F32)
    return jax.lax.dot_general(a, b, dims, preferred_element_type=_F32)


def _pack(p):
    return jnp.concatenate([
        pltpu.pack_elementwise([p[x:x + 8], p[x + 8:x + 16]], packed_dtype=_BF)
        for x in range(0, p.shape[0], 16)], axis=0)


def _kernel(x_hbm, wq_hbm, wk_hbm, wv_hbm, wo_hbm, w1_hbm, w2_hbm, w3_hbm, w4_hbm, o_ref,
            x_s, wq_s, wkv_s, wo_s, w1_s, w2_s, w3_s, w4_s,
            xn_s, xm_s, h_s, qe_s, qf_s, qn_s, kf_s, ke_s, kb_s, vt_s, ot_s, pv_s, sems):
    i = pl.program_id(0)
    nb = S // TQ

    def cp(n):
        src, dst = {
            "x0": (x_hbm.at[0, pl.ds(0 * TQ, TQ)], x_s.at[pl.ds(0 * TQ, TQ)]),
            "x1": (x_hbm.at[0, pl.ds(1 * TQ, TQ)], x_s.at[pl.ds(1 * TQ, TQ)]),
            "x2": (x_hbm.at[0, pl.ds(2 * TQ, TQ)], x_s.at[pl.ds(2 * TQ, TQ)]),
            "x3": (x_hbm.at[0, pl.ds(3 * TQ, TQ)], x_s.at[pl.ds(3 * TQ, TQ)]),
            "wk": (wk_hbm, wkv_s.at[pl.ds(0, DH)]),
            "wv": (wv_hbm, wkv_s.at[pl.ds(DH, DH)]),
            "wq": (wq_hbm, wq_s), "w1": (w1_hbm, w1_s), "w2": (w2_hbm, w2_s),
            "wo": (wo_hbm, wo_s), "w3": (w3_hbm, w3_s), "w4": (w4_hbm, w4_s),
        }[n]
        return pltpu.make_async_copy(src, dst, sems.at[names.index(n)])

    names = ["x0", "x1", "x2", "x3", "wq", "wk", "wv", "w1", "w2", "wo", "w3", "w4"]

    def norms(rows):
        xn = _ln(x_s[rows, :].astype(_F32))
        xn_s[rows, :] = xn.astype(_BF)
        xm_s[rows, :] = _ln(xn).astype(_BF)

    @pl.when(i == 0)
    def _prologue():
        for n in ("wq", "x0", "w1", "wk", "wv"):
            cp(n).start()
        h_s[pl.ds(0, PAD), :] = jnp.zeros((PAD, D), _F32)
        h_s[pl.ds(PAD + S, PAD), :] = jnp.zeros((PAD, D), _F32)
        cp("wq").wait()
        wqt = wq_s[...].T
        hsel = (jax.lax.broadcasted_iota(jnp.int32, (H, D), 1) // DH
                == jax.lax.broadcasted_iota(jnp.int32, (H, D), 0)).astype(_BF)
        cp("x0").wait()
        norms(pl.ds(0, TQ))
        cp("wk").wait()
        cp("wv").wait()
        cp("w1").wait()
        for n in ("x1", "x2", "x3"):
            cp(n).start()

        def block(b, kn):
            rows = pl.ds(pl.multiple_of(b * TQ, TQ), TQ)
            nxt = pl.ds(pl.multiple_of(jnp.minimum(b + 1, nb - 1) * TQ, TQ), TQ)

            @pl.when(b + 1 < nb)
            def _():
                pltpu.make_async_copy(x_hbm.at[0, nxt], x_s.at[nxt], sems.at[b + 1]).wait()

            xn = xn_s[rows, :]
            hpre = _dot(xm_s[rows, :], w1_s[...])
            kvt = _dot(wkv_s[...], xn, _NT).astype(_BF)
            qt = _dot(wqt, xn, _NT)
            h_s[pl.ds(pl.multiple_of(PAD + b * TQ, 8), TQ), :] = _gelu(hpre)
            vt_s[b] = kvt[DH:, :]
            kt = kvt[:DH, :].astype(_F32)
            kn = jnp.maximum(kn, jnp.sum(kt * kt, axis=0, keepdims=True))
            row = jax.lax.broadcasted_iota(jnp.int32, (2 * DH, TQ), 0)
            ket = jnp.where(row < DH, kvt.astype(_F32), jnp.where(row == DH, -1.0, 0.0))
            kf_s[...] = ket.T
            kp = jnp.concatenate([
                kf_s[pl.ds(e, TQ // 2, stride=2), :].reshape(TQ // 16, 8, 2 * DH) for e in range(2)],
                axis=1).reshape(TQ, 2 * DH)
            ke_s[pl.ds(pl.multiple_of(b * (TQ // 2), TQ // 2), TQ // 2), :] = pltpu.bitcast(kp.astype(_BF), jnp.uint32)
            qt = (qt * (DH ** -0.5 * math.log2(math.e))).astype(_BF)
            qf = qt.astype(_F32)
            for h in range(H):
                qe_s[b, pl.ds(2 * DH * h, DH), :] = qt[DH * h:DH * (h + 1), :]
                qf_s[b, h, pl.ds(0, DH), :] = qf[DH * h:DH * (h + 1), :]
            qn_s[b] = _dot(hsel, (qf * qf).astype(_BF))
            norms(nxt)
            return kn

        kn = jax.lax.fori_loop(0, nb, block, jnp.zeros((1, TQ), _F32))
        for n in ("w2", "wo", "w3", "w4"):
            cp(n).start()
        kmax = jnp.sqrt(jnp.max(kn, axis=1, keepdims=True)) * 1.02
        kv = pltpu.bitcast(ke_s[pl.ds((S - NV) // 2, NV // 2), :], _BF).astype(_F32)
        for d in range(DH):
            kb_s[d] = jnp.broadcast_to(kv[:, d:d + 1], (NV, 128))

        def bound(b, c):
            mh = (jnp.sqrt(qn_s[b]) * kmax).astype(_BF).astype(_F32)
            for h in range(H):
                qe_s[b, pl.ds(2 * DH * h + DH, DH), :] = jnp.broadcast_to(
                    mh[h:h + 1, :], (DH, TQ)).astype(_BF)
                qf_s[b, h, pl.ds(DH, 8), :] = jnp.broadcast_to(-mh[h:h + 1, :], (8, TQ))
            return c
        jax.lax.fori_loop(0, nb, bound, 0)

    nk = S // TK

    ns = (S - NV) // TS
    vwork = [(a, b) for a in range(0, NV, 16) for b in range(0, TQ, 128)]

    def vt(lo, hi):
        return vt_s[lo // TQ, :, lo % TQ:lo % TQ + hi - lo]

    def heads(g, ok):
        qts = [qe_s[i, pl.ds(pl.multiple_of((g * U + u) * 2 * DH, 2 * DH), 2 * DH), :] for u in range(U)]
        accs = [None] * U
        ls = [None] * U
        lv = [{} for _ in range(U)]
        scores, ready, back, pq = {}, {}, {}, []
        never = h_s[0:8, 0:128] > 0.5
        T = U * ns
        for t in range(T + LAG + PL):
            if t < T:
                u, j = divmod(t, ns)
                kw = ke_s[j * TS // 2:(j + 1) * TS // 2, :]
                if t in back:
                    kw = jnp.concatenate([jnp.where(never[:, :2 * DH], back.pop(t), kw[:8]), kw[8:]], axis=0)
                scores[t] = _dot(pltpu.bitcast(kw, _BF), qts[u])
            if t in ready:
                u, j, pp = ready.pop(t)
                e = (j + 1) * TS
                lo = e - 2 * pp.shape[0]
                if j == ns - 1:
                    pp, e = jnp.concatenate([pp, pv_s[u % 2]], axis=0), S
                a = _dot(vt(lo, e), pltpu.bitcast(pp, _BF))
                accs[u] = a if accs[u] is None else accs[u] + a
                if j == ns - 1:
                    acc = accs[u]
                    l = ls[u] + jnp.concatenate([lv[u][b] for b in range(0, TQ, 128)], axis=1)
                    l = jnp.sum(l, axis=0, keepdims=True)
                    ok = jnp.where((l >= L_SAFE) & (l <= 2.0 * S), ok, 0.0)
                    ot_s[pl.ds(pl.multiple_of((g * U + u) * DH, DH), DH), :] = (
                        acc * (1.0 / l)).astype(_BF)
            if LAG <= t < T + LAG:
                u, j = divmod(t - LAG, ns)
                sc = scores.pop(t - LAG)
                p = jnp.exp2(sc)
                ps = p.reshape(TS // 8, 8, TQ).sum(axis=0)
                ls[u] = ps if ls[u] is None else ls[u] + ps
                pq.append(_pack(p))
                if len(pq) == TP // TS or j == ns - 1:
                    ready[t + PL] = (u, j, jnp.concatenate(pq, axis=0))
                    pq = []
                for a, b in vwork[j * len(vwork) // ns:(j + 1) * len(vwork) // ns]:
                    hq = g * U + u
                    sv = jnp.where(never, sc[:8, b:b + 128], qf_s[i, hq, DH:DH + 8, b:b + 128])
                    sv = jnp.concatenate([sv, sv], axis=0)
                    for d in range(DH):
                        sv = sv + kb_s[d, a:a + 16, :] * jnp.broadcast_to(
                            qf_s[i, hq, d:d + 1, b:b + 128], (16, 128))
                    p = jnp.exp2(sv)
                    ps = p[:8] + p[8:]
                    lv[u][b] = lv[u][b] + ps if b in lv[u] else ps
                    pw = _pack(p)
                    pv_s[u % 2, a // 2:a // 2 + 8, b:b + 128] = pw
                    back[t - LAG + W] = pw[:, :2 * DH]
        return ok

    ok = jax.lax.fori_loop(0, H // U, heads, jnp.ones((1, TQ), _F32))

    @pl.when(jnp.min(ok) < 0.5)
    def _fallback():
        def head(h, c):
            qt = qe_s[i, pl.ds(pl.multiple_of(h * 2 * DH, 2 * DH), DH), :]

            def chunk(j, carry):
                m, l, acc = carry
                r = pl.ds(pl.multiple_of(j * (TK // 2), TK // 2), TK // 2)
                s = _dot(pltpu.bitcast(ke_s[r, :], _BF)[:, :DH], qt)
                mn = jnp.maximum(m, jnp.max(s, axis=0, keepdims=True))
                p = jnp.exp2(s - mn)
                a = jnp.exp2(m - mn)
                l = a * l + jnp.sum(p, axis=0, keepdims=True)
                acc = a * acc + _dot(vt_s[j], pltpu.bitcast(_pack(p), _BF))
                return mn, l, acc

            m, l, acc = jax.lax.fori_loop(
                0, nk, chunk,
                (jnp.full((1, TQ), -jnp.inf, _F32), jnp.zeros((1, TQ), _F32), jnp.zeros((DH, TQ), _F32)))
            ot_s[pl.ds(pl.multiple_of(h * DH, DH), DH), :] = (acc / l).astype(_BF)
            return c
        jax.lax.fori_loop(0, H, head, 0)

    @pl.when(i == 0)
    def _():
        cp("w2").wait()
        cp("wo").wait()
        cp("w3").wait()
        cp("w4").wait()

    c = D // 4
    TM = TQ // NS
    parts = range(NS)
    rows = [pl.ds(pl.multiple_of(i * TQ + r * TM, TM), TM) for r in parts]

    def shifted(r):
        hw = h_s[pl.ds(pl.multiple_of(i * TQ + r * TM, TM), TM + 2 * PAD), :]
        return jnp.concatenate([
            hw[PAD - 1:PAD - 1 + TM, 0 * c:1 * c],
            hw[PAD + 1:PAD + 1 + TM, 1 * c:2 * c],
            hw[PAD - 2:PAD - 2 + TM, 2 * c:3 * c],
            hw[PAD + 2:PAD + 2 + TM, 3 * c:4 * c]], axis=1).astype(_BF)

    def attn_out(r):
        return _dot(ot_s[:, r * TM:(r + 1) * TM], wo_s[...], _TN)

    x1 = [xn_s[rows[r], :].astype(_F32) + _dot(shifted(r), w2_s[...]) for r in parts]
    sattn = [attn_out(r) for r in range(NS - 1)]
    up = [_dot(_ln(x1[r]).astype(_BF), w3_s[...]) for r in parts]
    z = [x1[r] + _dot(_gelu(up[r]).astype(_BF), w4_s[...]) for r in parts]
    sattn.append(attn_out(NS - 1))
    for r in parts:
        gate = z[r] * (1.0 / (1.0 + jnp.exp(-z[r])))
        o_ref[0, r * TM:(r + 1) * TM, :] = (
            x_s[rows[r], :].astype(_F32) + sattn[r] * gate).astype(o_ref.dtype)


@jax.jit
def pallas_recurrent_scan__grouped_kv_mqa__mixer_s_mlp__prompt_kernel(
        A_x, A_wq, A_wk, A_wv, A_wo, B_x, B_w1, B_w2, B_w3, B_w4):
    any_spec = pl.BlockSpec(memory_space=pl.ANY)
    return pl.pallas_call(
        _kernel,
        grid=(S // TQ,),
        in_specs=[any_spec] * 9,
        out_specs=pl.BlockSpec((1, TQ, D), lambda i: (0, i, 0)),
        out_shape=jax.ShapeDtypeStruct((1, S, D), A_x.dtype),
        scratch_shapes=[
            pltpu.VMEM((S, D), _BF), pltpu.VMEM((D, D), _BF), pltpu.VMEM((2 * DH, D), _BF),
            pltpu.VMEM((D, D), _BF), pltpu.VMEM((D, D), _BF), pltpu.VMEM((D, D), _BF),
            pltpu.VMEM((D, F), _BF), pltpu.VMEM((F, D), _BF),
            pltpu.VMEM((S, D), _BF), pltpu.VMEM((S, D), _BF), pltpu.VMEM((S + 2 * PAD, D), _F32),
            pltpu.VMEM((S // TQ, 2 * DH * H, TQ), _BF), pltpu.VMEM((S // TQ, H, DH + 8, TQ), _F32),
            pltpu.VMEM((S // TQ, H, TQ), _F32), pltpu.VMEM((TQ, 2 * DH), _F32),
            pltpu.VMEM((S // 2, 2 * DH), jnp.uint32), pltpu.VMEM((DH, NV, 128), _F32),
            pltpu.VMEM((S // TQ, DH, TQ), _BF), pltpu.VMEM((D, TQ), _BF),
            pltpu.VMEM((2, NV // 2, TQ), jnp.uint32),
            pltpu.SemaphoreType.DMA((12,)),
        ],
        compiler_params=pltpu.CompilerParams(
            dimension_semantics=("arbitrary",), vmem_limit_bytes=100 * 2 ** 20),
    )(A_x, A_wq, A_wk.T, A_wv.T, A_wo, B_w1, B_w2, B_w3, B_w4)
```
